```python
import jax
import jax.numpy as jnp

def _softmax(x, axis=-1):
    return jax.nn.softmax(x, axis=axis)

def _gelu(x):
    return jax.nn.gelu(x, approximate=True)

def _silu(x):
    return jax.nn.silu(x)

def _sigmoid(x):
    return jax.nn.sigmoid(x)

def _layernorm(x, axis=-1, eps=1e-05):
    m = jnp.mean(x, axis=axis, keepdims=True)
    v = jnp.var(x, axis=axis, keepdims=True)
    return (x - m) / jnp.sqrt(v + eps)

def _scatter_add(tgt, idx, src, axis=0):
    return tgt.at[idx].add(src)

def _segment_sum(src, seg, n):
    return jax.ops.segment_sum(src, seg, n)

class _Rng:

    def __init__(self, key):
        self._k = key

    def _next(self):
        self._k, sub = jax.random.split(self._k)
        return sub

    def normal(self, shape):
        return jax.random.normal(self._next(), shape, dtype=jnp.bfloat16)

    def randint(self, lo, hi, shape):
        return jax.random.randint(self._next(), shape, lo, hi, dtype=jnp.int32)

    def uniform(self, shape, lo=0.0, hi=1.0):
        return jax.random.uniform(self._next(), shape, jnp.bfloat16, lo, hi)

    def permutation(self, n):
        return jax.random.permutation(self._next(), n)
kernel_name = 'recurrent_scan__ssm_conv_h3__mixer_gmlp__prompt'

def setup_inputs():
    _rng = _Rng(jax.random.key(int.from_bytes(__import__("os").urandom(4), "little")))
    _w = lambda a: (lambda t: t.astype(jnp.bfloat16) if jnp.issubdtype(t.dtype, jnp.floating) else t)(jnp.asarray(a))

    def _A_setup():
        B, S, D = (1, 2048, 640)
        ks = 4
        return {'q': _w((lambda *s: _rng.normal(s) * 0.05)(B, S, D)), 'k': _w((lambda *s: _rng.normal(s) * 0.05)(B, S, D)), 'v': _w((lambda *s: _rng.normal(s) * 0.05)(B, S, D)), 'shift_k': _w((lambda *s: _rng.normal(s) * 0.05)(D, ks) * 0.5), 'ssm_k': _w((lambda *s: _rng.normal(s) * 0.05)(D, S) * (1.0 / S ** 0.5)), 'ssm_D': _w((lambda *s: _rng.normal(s) * 0.05)(D))}
    _A_in = _A_setup()

    def _B_setup():
        B, S, D, F = (1, 2048, 640, 1536)
        Fh = F // 2
        return {'x': _w((lambda *s: _rng.normal(s) * 0.05)(B, S, D)), 'w_in': _w((lambda *s: _rng.normal(s) * 0.05)(D, 2 * Fh)), 'w_sp': _w(0.01 * (lambda *s: _rng.normal(s) * 0.05)(S, S)), 'b_sp': _w(1.0 + 0.01 * (lambda *s: _rng.normal(s) * 0.05)(S)), 'w_out': _w((lambda *s: _rng.normal(s) * 0.05)(Fh, D))}
    _B_in = _B_setup()
    return {'A_q': _A_in['q'], 'A_k': _A_in['k'], 'A_v': _A_in['v'], 'A_shift_k': _A_in['shift_k'], 'A_ssm_k': _A_in['ssm_k'], 'A_ssm_D': _A_in['ssm_D'], 'B_x': _B_in['x'], 'B_w_in': _B_in['w_in'], 'B_w_sp': _B_in['w_sp'], 'B_b_sp': _B_in['b_sp'], 'B_w_out': _B_in['w_out']}

def reference(A_q, A_k, A_v, A_shift_k, A_ssm_k, A_ssm_D, B_x, B_w_in, B_w_sp, B_b_sp, B_w_out):

    def _A_ref(q, k, v, shift_k, ssm_k, ssm_D):
        B, S, D = q.shape
        ks = shift_k.shape[-1]
        k_pad = jnp.pad(k, ((0, 0), (ks - 1, 0), (0, 0)))
        k_shift = jnp.zeros_like(k)
        for t in range(ks):
            k_shift = k_shift + k_pad[:, t:t + S, :] * shift_k[:, ks - 1 - t][None, None, :]
        kv = k_shift * v
        L = 2 * S
        kv_pad = jnp.pad(kv, ((0, 0), (0, S), (0, 0)))
        kf_pad = jnp.pad(ssm_k, ((0, 0), (0, S)))
        kv_f = (lambda x, axes=(-2, -1): jnp.fft.rfft2(x.astype(jnp.float32), axes=axes))(kv_pad[:, None, :, :], axes=(1, 2))
        kf_f = (lambda x, axes=(-2, -1): jnp.fft.rfft2(x.astype(jnp.float32), axes=axes))(kf_pad[:, None, :], axes=(1, 2))
        kf_f = (lambda x, *d: x.transpose(*d))(kf_f, 1, 2, 0)
        y_f = kv_f * kf_f[None, :, :, :]
        y = (lambda x, s, axes=(-2, -1): jnp.fft.irfft2(x, s=s, axes=axes).astype(jnp.bfloat16))(y_f, (1, L), axes=(1, 2))[:, 0, :S, :]
        y = y + kv * ssm_D[None, None, :]
        return q * y

    def _B_ref(x, w_in, w_sp, b_sp, w_out):
        B, S, D = x.shape
        F = w_in.shape[-1]
        Fh = F // 2
        z = _gelu(jnp.einsum('bsd,df->bsf', x, w_in))
        z1 = z[..., :Fh].copy()
        z2 = _layernorm(z[..., Fh:], axis=-1)
        g = jnp.einsum('ts,bsf->btf', w_sp, z2) + b_sp[None, :, None]
        return jnp.einsum('bsf,fd->bsd', z1 * g, w_out)
    x = A_q
    xn = _layernorm(x, axis=-1)
    s = _A_ref(xn, A_k, A_v, A_shift_k, A_ssm_k, A_ssm_D)
    g = _silu(_B_ref(xn, B_w_in, B_w_sp, B_b_sp, B_w_out))
    return x + s * g
```

```python
import functools

import jax
import jax.numpy as jnp
import numpy as np
from jax import lax
import jax.experimental.pallas as pl
import jax.experimental.pallas.tpu as pltpu

S, D, F, FH, KS = 2048, 640, 1536, 768, 4
C = 128
NC = S // C
TB = 256
NB = S // TB
CPB = TB // C
CG = D // NB
HALO = 16
EPS = 1e-5


def _dft_mats():
    t = np.arange(C, dtype=np.float64)[:, None]
    w = 2.0 * np.pi * (np.arange(C, dtype=np.float64)[None, :] + 0.5) / (2 * C)
    fwd = np.concatenate([np.cos(w * t), -np.sin(w * t)], axis=1)
    inv = fwd.T / C
    return fwd.astype(np.float32), inv.astype(np.float32)


def _layernorm(x):
    m = jnp.mean(x, axis=-1, keepdims=True)
    xc = x - m
    v = jnp.mean(xc * xc, axis=-1, keepdims=True)
    return xc * lax.rsqrt(v + EPS)


def _gelu(x):
    c0 = np.float32(np.sqrt(2.0 / np.pi))
    c1 = np.float32(np.sqrt(2.0 / np.pi) * 0.044715)
    return (0.5 * x) * (1.0 + jnp.tanh(x * (c0 + c1 * (x * x))))


def _kernel(x_hbm, k_hbm, v_hbm, shk_ref, ssmk_hbm, d_ref, win_hbm, wsp_hbm, b_ref,
            wout_hbm, wf_ref, wi_ref, out_hbm,
            x_s, k_s, v_s, ssmk_s, win_s, wsp_s, wout_s, xn_s, kv_s, z1_s, z2_s,
            u_s, kf_s, z_s, kprev_s, b_s, out_s, sem_in, sem_k, sem_w, sem_out):
    f32, bf16 = jnp.float32, jnp.bfloat16

    def rows(p):
        return pl.ds(pl.multiple_of(p * TB, TB), TB)

    def cp_x(p):
        return pltpu.make_async_copy(x_hbm.at[rows(p)], x_s.at[rows(p)], sem_in.at[0, p])

    def cp_k(p):
        return pltpu.make_async_copy(
            k_hbm.at[rows(p)],
            k_s.at[pl.ds(pl.multiple_of(p * TB + HALO, HALO), TB)], sem_in.at[1, p])

    def cp_v(p):
        return pltpu.make_async_copy(v_hbm.at[rows(p)], v_s.at[rows(p)], sem_in.at[2, p])

    def cp_wsp(p):
        return pltpu.make_async_copy(wsp_hbm.at[rows(p)], wsp_s.at[rows(p)], sem_in.at[3, p])

    def cp_ssmk(m):
        return pltpu.make_async_copy(
            ssmk_hbm.at[:, pl.ds(pl.multiple_of(m * C, C), C)], ssmk_s.at[m], sem_k.at[m])

    def cp_out(p):
        return pltpu.make_async_copy(out_s.at[rows(p)], out_hbm.at[rows(p)], sem_out.at[p])

    cp_win = pltpu.make_async_copy(win_hbm, win_s, sem_w.at[0])
    cp_wout = pltpu.make_async_copy(wout_hbm, wout_s, sem_w.at[1])

    def start_block(p):
        cp_x(p).start()
        cp_k(p).start()
        cp_v(p).start()
        for c in range(CPB):
            cp_ssmk(p * CPB + c).start()

    cp_win.start()
    start_block(0)
    start_block(1)

    k_s[pl.ds(0, HALO), :] = jnp.zeros((HALO, D), bf16)
    kprev_s[...] = jnp.zeros((D, 2 * C), f32)
    for c in range(NC):
        brow = b_ref[:, c * C:(c + 1) * C].astype(f32)
        b_s[c * C:(c + 1) * C, :] = jnp.broadcast_to(brow, (C, C)).T
    lane = lax.broadcasted_iota(jnp.int32, (1, C), 1)
    sgn = (1 - 2 * (lane & 1)).astype(f32)

    cp_win.wait()

    def phase1(p, carry):
        @pl.when(p + 2 < NB)
        def _():
            start_block(p + 2)
        cp_wsp(p).start()

        @pl.when(p == 0)
        def _():
            cp_wout.start()

        cp_x(p).wait()
        cp_k(p).wait()
        cp_v(p).wait()
        for c in range(CPB):
            cp_ssmk(p * CPB + c).wait()

        r = rows(p)
        xn = _layernorm(x_s[r, :].astype(f32)).astype(bf16)
        xn_s[r, :] = xn
        z1 = _gelu(jnp.dot(xn, win_s[:, :FH], preferred_element_type=f32))
        z1_s[r, :] = z1.astype(bf16)
        z2 = _gelu(jnp.dot(xn, win_s[:, FH:], preferred_element_type=f32))
        z2_s[r, :] = _layernorm(z2).astype(bf16)

        kwin = k_s[pl.ds(pl.multiple_of(p * TB, HALO), TB + HALO), :].astype(f32)
        shk = shk_ref[...].astype(f32)
        ksh = kwin[HALO:, :] * shk[0:1, :]
        for tau in range(1, KS):
            ksh = ksh + kwin[HALO - tau:HALO - tau + TB, :] * shk[tau:tau + 1, :]
        kv = ksh * v_s[r, :].astype(f32)
        kv_s[r, :] = kv.astype(bf16)
        parts = [kv[c * C:(c + 1) * C, :].T.astype(bf16) for c in range(CPB)]
        parts += [ssmk_s[p * CPB + c] for c in range(CPB)]
        spec = jnp.dot(jnp.concatenate(parts, axis=0), wf_ref[...],
                       preferred_element_type=f32)
        for c in range(CPB):
            u_s[p * CPB + c] = spec[c * D:(c + 1) * D, :]
        prev = kprev_s[...]
        for c in range(CPB):
            cur = spec[(CPB + c) * D:(CPB + c + 1) * D, :]
            kf_s[p * CPB + c, :, :C] = cur[:, :C] - sgn * prev[:, C:]
            kf_s[p * CPB + c, :, C:] = cur[:, C:] + sgn * prev[:, :C]
            prev = cur
        kprev_s[...] = prev
        return carry

    lax.fori_loop(0, NB, phase1, 0)

    IB = 4

    def phase2(p, carry):
        cp_wsp(p).wait()
        r = rows(p)
        g = jnp.dot(wsp_s[r, :], z2_s[...], preferred_element_type=f32)
        g = g + jnp.tile(b_s[r, :], (1, FH // C))
        z1_s[r, :] = (z1_s[r, :].astype(f32) * g).astype(bf16)

        for gi in range(CG // 8):
            ch = pl.ds(pl.multiple_of(p * CG + gi * 8, 8), 8)
            for ib in range(0, NC, IB):
                ucache = {}
                accr = [None] * IB
                acci = [None] * IB
                for m in range(ib + IB):
                    kr = kf_s[m, ch, :C]
                    ki = kf_s[m, ch, C:]
                    for q in range(IB):
                        j = ib + q - m
                        if j < 0:
                            continue
                        if j not in ucache:
                            ucache[j] = (u_s[j, ch, :C], u_s[j, ch, C:])
                        ur, ui = ucache[j]
                        pr = kr * ur - ki * ui
                        pi = kr * ui + ki * ur
                        accr[q] = pr if accr[q] is None else accr[q] + pr
                        acci[q] = pi if acci[q] is None else acci[q] + pi
                for q in range(IB):
                    z_s[ib + q, ch, :C] = accr[q]
                    z_s[ib + q, ch, C:] = acci[q]
        return carry

    lax.fori_loop(0, NB, phase2, 0)

    cp_wout.wait()

    def phase3(p, carry):
        r = rows(p)
        o = jnp.dot(z1_s[r, :], wout_s[...], preferred_element_type=f32)
        gate = o * jax.nn.sigmoid(o)
        zb = jnp.concatenate([z_s[p * CPB + c].astype(bf16) for c in range(CPB)], axis=0)
        yt = jnp.dot(zb, wi_ref[...], preferred_element_type=f32)
        y = jnp.concatenate([yt[c * D:(c + 1) * D, :].T for c in range(CPB)], axis=0)
        y = y + kv_s[r, :].astype(f32) * d_ref[...].astype(f32)
        s = xn_s[r, :].astype(f32) * y
        out_s[r, :] = (x_s[r, :].astype(f32) + s * gate).astype(bf16)
        cp_out(p).start()
        return carry

    lax.fori_loop(0, NB, phase3, 0)
    for p in range(NB):
        cp_out(p).wait()


@jax.jit
def pallas_recurrent_scan__ssm_conv_h3__mixer_gmlp__prompt_kernel(
    A_q: jax.Array,
    A_k: jax.Array,
    A_v: jax.Array,
    A_shift_k: jax.Array,
    A_ssm_k: jax.Array,
    A_ssm_D: jax.Array,
    B_x: jax.Array,
    B_w_in: jax.Array,
    B_w_sp: jax.Array,
    B_b_sp: jax.Array,
    B_w_out: jax.Array,
):
    del B_x
    f32, bf16 = jnp.float32, jnp.bfloat16
    wf, wi = _dft_mats()
    hbm = pl.BlockSpec(memory_space=pl.ANY)
    vmem = pl.BlockSpec(memory_space=pltpu.VMEM)
    out = pl.pallas_call(
        _kernel,
        out_shape=jax.ShapeDtypeStruct((S, D), bf16),
        in_specs=[hbm, hbm, hbm, vmem, hbm, vmem, hbm, hbm, vmem, hbm, vmem, vmem],
        out_specs=hbm,
        scratch_shapes=[
            pltpu.VMEM((S, D), bf16),
            pltpu.VMEM((S + HALO, D), bf16),
            pltpu.VMEM((S, D), bf16),
            pltpu.VMEM((NC, D, C), bf16),
            pltpu.VMEM((D, F), bf16),
            pltpu.VMEM((S, S), bf16),
            pltpu.VMEM((FH, D), bf16),
            pltpu.VMEM((S, D), bf16),
            pltpu.VMEM((S, D), bf16),
            pltpu.VMEM((S, FH), bf16),
            pltpu.VMEM((S, FH), bf16),
            pltpu.VMEM((NC, D, 2 * C), f32),
            pltpu.VMEM((NC, D, 2 * C), f32),
            pltpu.VMEM((NC, D, 2 * C), f32),
            pltpu.VMEM((D, 2 * C), f32),
            pltpu.VMEM((S, C), f32),
            pltpu.VMEM((S, D), bf16),
            pltpu.SemaphoreType.DMA((4, NB)),
            pltpu.SemaphoreType.DMA((NC,)),
            pltpu.SemaphoreType.DMA((2,)),
            pltpu.SemaphoreType.DMA((NB,)),
        ],
        compiler_params=pltpu.CompilerParams(vmem_limit_bytes=100 * 1024 * 1024),
    )(
        A_q.reshape(S, D), A_k.reshape(S, D), A_v.reshape(S, D),
        A_shift_k.T, A_ssm_k, A_ssm_D.reshape(1, D), B_w_in, B_w_sp,
        B_b_sp.reshape(1, S), B_w_out,
        jnp.asarray(wf, dtype=bf16), jnp.asarray(wi, dtype=bf16),
    )
    return out.reshape(1, S, D)
```

```python
import functools

import jax
import jax.numpy as jnp
import numpy as np
from jax import lax
import jax.experimental.pallas as pl
import jax.experimental.pallas.tpu as pltpu

S, D, F, FH, KS = 2048, 640, 1536, 768, 4
C = 128
NC = S // C
TB = 256
NB = S // TB
CPB = TB // C
CG = D // NB
HALO = 16
EPS = 1e-5


def _dft_mats():
    t = np.arange(C, dtype=np.float64)[:, None]
    w = 2.0 * np.pi * (np.arange(C, dtype=np.float64)[None, :] + 0.5) / (2 * C)
    fwd = np.concatenate([np.cos(w * t), -np.sin(w * t)], axis=1)
    inv = fwd.T / C
    return fwd.astype(np.float32), inv.astype(np.float32)


def _layernorm(x):
    m = jnp.mean(x, axis=-1, keepdims=True)
    xc = x - m
    v = jnp.mean(xc * xc, axis=-1, keepdims=True)
    return xc * lax.rsqrt(v + EPS)


def _gelu(x):
    c0 = np.float32(np.sqrt(2.0 / np.pi))
    c1 = np.float32(np.sqrt(2.0 / np.pi) * 0.044715)
    return (0.5 * x) * (1.0 + jnp.tanh(x * (c0 + c1 * (x * x))))


def _pk(v):
    return pltpu.bitcast(v, jnp.uint32)


def _unpk(u):
    return pltpu.bitcast(u, jnp.bfloat16)


def _run_schedule(main, sides):
    done = [0] * len(sides)
    for u, f in enumerate(main):
        f()
        for si, (pieces, u0, u1) in enumerate(sides):
            n = len(pieces)
            tgt = n if u >= u1 - 1 else max(0, (u - u0 + 1) * n // (u1 - u0))
            while done[si] < tgt:
                pieces[done[si]]()
                done[si] += 1


def _kernel(x_hbm, k_hbm, v_hbm, shk_ref, ssmk_hbm, d_ref, win_hbm, wsp_hbm, b_ref,
            wout_hbm, wf_ref, wi_ref, out_hbm,
            x_s, k_s, v_s, ssmk_s, wsp_s, wout_s, xn_s, kv_s, z1_s, z2_s,
            u_s, kf_s, b_s, acc_s, kvt_s, zb_s, h_s, y_s, gate_s, winp_s, wfp_s, wip_s, kvb0_s, out_s, go_s, sem_in, sem_k, sem_w, sem_out):
    f32, bf16 = jnp.float32, jnp.bfloat16

    u32 = jnp.uint32
    wsp_hbm, win_hbm = wsp_hbm.bitcast(u32), win_hbm.bitcast(u32)
    wout_hbm, ssmk_hbm = wout_hbm.bitcast(u32), ssmk_hbm.bitcast(u32)

    def rows(p):
        return pl.ds(pl.multiple_of(p * TB, TB), TB)

    def cp_x(p):
        return pltpu.make_async_copy(x_hbm.at[rows(p)], x_s.at[rows(p)], sem_in.at[0, p])

    def cp_k(p):
        return pltpu.make_async_copy(
            k_hbm.at[rows(p)],
            k_s.at[pl.ds(pl.multiple_of(p * TB + HALO, HALO), TB)], sem_in.at[1, p])

    def cp_v(p):
        return pltpu.make_async_copy(v_hbm.at[rows(p)], v_s.at[rows(p)], sem_in.at[2, p])

    def cp_wsp(p):
        r = pl.ds(pl.multiple_of(p * (TB // 2), TB // 2), TB // 2)
        return pltpu.make_async_copy(wsp_hbm.at[r], wsp_s.at[r], sem_in.at[3, p])

    def cp_ssmk(m):
        return pltpu.make_async_copy(
            ssmk_hbm.at[:, pl.ds(pl.multiple_of(m * C, C), C)], ssmk_s.at[m], sem_k.at[m])

    def cp_out(p):
        return pltpu.make_async_copy(out_s.at[rows(p)], out_hbm.at[rows(p)], sem_out.at[p])

    cp_win = [pltpu.make_async_copy(win_hbm.at[:, FH:], winp_s.at[:, :FH], sem_w.at[0]),
              pltpu.make_async_copy(win_hbm.at[:, :FH], winp_s.at[:, FH:], sem_w.at[2])]
    cp_wout = pltpu.make_async_copy(wout_hbm, wout_s, sem_w.at[1])

    def start_kv(p):
        cp_k(p).start()
        cp_v(p).start()
        for c in range(CPB):
            cp_ssmk(p * CPB + c).start()

    cp_x(0).start()
    for cp in cp_win:
        cp.start()

    go_s[0] = 1
    k_s[pl.ds(0, HALO), :] = jnp.zeros((HALO, D), bf16)
    for c in range(NC):
        brow = b_ref[:, c * C:(c + 1) * C].astype(f32)
        b_s[c * C:(c + 1) * C, :] = jnp.broadcast_to(brow, (C, C)).T

    def rws(p, off, n):
        return pl.ds(pl.multiple_of(p * TB + off, n if n < 16 else 16), n)

    def hrws(p, off, n):
        return pl.ds(pl.multiple_of((p * TB + off) // 2, 8), n // 2)

    def ln_piece(p, i):
        def f():
            r = rws(p, 16 * i, 16)
            xn_s[hrws(p, 16 * i, 16), :] = _pk(_layernorm(x_s[r, :].astype(f32)).astype(bf16))
        return f

    CONV_N = 64

    def conv_piece(p, dst, i, t):
        def f():
            n = CONV_N
            cs = slice(t * C, (t + 1) * C)
            shk = shk_ref[:, cs].astype(f32)
            kwin = k_s[pl.ds(pl.multiple_of(p * TB + HALO + n * i - 8, 8), n + 8), cs].astype(f32)
            ksh = kwin[8:, :] * shk[0:1, :]
            for tau in range(1, KS):
                ksh = ksh + kwin[8 - tau:8 - tau + n, :] * shk[tau:tau + 1, :]
            r = rws(p, n * i, n)
            kv = ksh * v_s[r, cs].astype(f32)
            kv_s[r, cs] = kv.astype(bf16)
            dst[n * i:n * (i + 1), cs] = kv
        return f

    def tr_piece(src, slot, c, t):
        def f():
            blk = src[c * C:(c + 1) * C, t * C:(t + 1) * C]
            kvt_s[slot, c, t * C // 2:(t + 1) * C // 2, :] = _pk(blk.T.astype(bf16))
        return f

    wfp_s[...] = _pk(wf_ref[...])
    wip_s[...] = _pk(wi_ref[...])

    kvt_s[...] = jnp.zeros((2, CPB, D // 2, C), jnp.uint32)
    cp_x(0).wait()
    cp_x(1).start()
    for i in range(TB // 16):
        ln_piece(0, i)()
    for cp in cp_win:
        cp.wait()

    MB = 64
    MQ = TB // MB
    NG = 4 * C

    def phase1_body(p):
        pn = jnp.minimum(p + 1, NB - 1)

        def mm1_a(j, mq, t):
            def f():
                cs = slice(j * NG + t * C, j * NG + (t + 1) * C)
                d = jnp.dot(_unpk(xn_s[hrws(p, mq * MB, MB), :4 * C]), _unpk(winp_s[:2 * C, cs]),
                            preferred_element_type=f32)
                acc_s[mq * MB:(mq + 1) * MB, cs] = d
            return f

        def mm1_b(j, mq):
            def f():
                cs = slice(j * NG, (j + 1) * NG)
                d = jnp.dot(_unpk(xn_s[hrws(p, mq * MB, MB), 4 * C:]), _unpk(winp_s[2 * C:, cs]),
                            preferred_element_type=f32)
                acc_s[mq * MB:(mq + 1) * MB, cs] += d
            return f

        def gelu_piece(j, mq, t):
            def f():
                c0 = j * NG + t * C
                rs = slice(mq * MB, (mq + 1) * MB)
                z = _gelu(acc_s[rs, c0:c0 + C])
                if c0 < FH:
                    acc_s[rs, c0:c0 + C] = z
                else:
                    z1_s[hrws(p, mq * MB, MB), c0 - FH:c0 - FH + C] = _pk(z.astype(bf16))
            return f

        def ln2_piece(i):
            def f():
                z2 = acc_s[16 * i:16 * (i + 1), :FH]
                z2_s[hrws(p, 16 * i, 16), :] = _pk(_layernorm(z2).astype(bf16))
            return f

        main = []
        for j in range(F // NG):
            for mq in range(MQ):
                main += [mm1_a(j, mq, t) for t in range(NG // C)] + [mm1_b(j, mq)]
        n_mm = len(main)
        upb = NG // C + 1
        sides = []
        for b in range(3 * MQ):
            j, mq = divmod(b, MQ)
            if b + 1 < 3 * MQ:
                sides.append(([gelu_piece(j, mq, t) for t in range(NG // C)],
                              (b + 1) * upb, (b + 2) * upb))
        sides.append(([ln2_piece(i) for i in range(TB // 16)], 45, 60))
        sides.append(([ln_piece(pn, i) for i in range(TB // 16)], 10, 40))
        _run_schedule(main, sides)
        for t in range(NG // C):
            gelu_piece(F // NG - 1, MQ - 1, t)()

    def phase1(p, carry):
        start_kv(p)

        @pl.when(p + 2 < NB)
        def _():
            cp_x(p + 2).start()
        cp_wsp(p).start()

        @pl.when(p == 0)
        def _():
            cp_wout.start()

        @pl.when(p + 1 < NB)
        def _():
            cp_x(p + 1).wait()
        pl.when(go_s[0] > 0)(functools.partial(phase1_body, p))
        return carry

    lax.fori_loop(0, NB, phase1, 0)

    def dft_unit(src, dst, blk, c, cb):
        def f():
            dst[blk * CPB + c, cb * C:(cb + 1) * C, :] = jnp.dot(
                _unpk(src(c, slice(cb * C // 2, (cb + 1) * C // 2))), _unpk(wfp_s[...]),
                preferred_element_type=f32)
        return f

    def u_units(blk, c):
        return [dft_unit(lambda c_, hr: kvt_s[0, c_, hr, :], u_s, blk, c, cb) for cb in range(D // C)]

    def phaseA_body(p):
        main = [dft_unit(lambda c_, hr: ssmk_s[p * CPB + c_, hr, :], kf_s, p, c, cb)
                for c in range(CPB) for cb in range(D // C)]
        main += u_units(p, 0) + u_units(p, 1)
        hc = C // CONV_N
        sides = []
        for c in range(CPB):
            sides.append(([conv_piece(p, kvb0_s, i, t) for t in range(D // C) for i in range(c * hc, (c + 1) * hc)],
                          5 * c, 5 * c + 5))
            sides.append(([tr_piece(kvb0_s, 0, c, t) for t in range(D // C)], 5 * c + 2, 5 * c + 8))
        _run_schedule(main, sides)

    def phaseA(p, carry):
        cp_k(p).wait()
        cp_v(p).wait()
        for c in range(CPB):
            cp_ssmk(p * CPB + c).wait()
        pl.when(go_s[0] > 0)(functools.partial(phaseA_body, p))
        return carry

    lax.fori_loop(0, NB, phaseA, 0)
    cp_wout.wait()

    IB = 4

    lane = lax.broadcasted_iota(jnp.int32, (1, C), 1)
    sgn = (1 - 2 * (lane & 1)).astype(f32)

    def mac_gen(p):
        for g2 in range(CG // 16):
            prev = [None, None]
            for ib in range(0, NC, IB):
                res = []
                for half in range(2):
                    ch = pl.ds(pl.multiple_of(p * CG + g2 * 16 + half * 8, 8), 8)
                    ucache = {}
                    accr = [None] * IB
                    acci = [None] * IB
                    for m in range(ib + IB):
                        kr = kf_s[m, ch, :C]
                        ki = kf_s[m, ch, C:]
                        for q in range(IB):
                            j = ib + q - m
                            if j < 0:
                                continue
                            if j not in ucache:
                                ucache[j] = (u_s[j, ch, :C], u_s[j, ch, C:])
                            ur, ui = ucache[j]
                            pr = kr * ur - ki * ui
                            pi = kr * ui + ki * ur
                            accr[q] = pr if accr[q] is None else accr[q] + pr
                            acci[q] = pi if acci[q] is None else acci[q] + pi
                            yield
                    out = []
                    for q in range(IB):
                        if prev[half] is None:
                            out.append((accr[q], acci[q]))
                        else:
                            out.append((accr[q] - sgn * prev[half][1], acci[q] + sgn * prev[half][0]))
                        prev[half] = (accr[q], acci[q])
                    res.append(out)
                ro = pl.ds(pl.multiple_of((p * CG + g2 * 16) // 2, 8), 8)
                for q in range(IB):
                    for part in range(2):
                        v = jnp.concatenate([res[0][q][part], res[1][q][part]], axis=0)
                        zb_s[ib + q, ro, part * C:(part + 1) * C] = _pk(v.astype(bf16))

    MB2 = 128
    MQ2 = TB // MB2

    def phase2_body(p):
        KQ = 4
        KW = S // KQ
        gen = mac_gen(p)

        def mm2(mq, n, kq):
            def f():
                cs = slice(n * C, (n + 1) * C)
                r = rws(p, mq * MB2, MB2)
                gr = slice(mq * MB2, (mq + 1) * MB2)
                ks = slice(kq * KW, (kq + 1) * KW)
                d = jnp.dot(_unpk(wsp_s[hrws(p, mq * MB2, MB2), ks]), _unpk(z2_s[kq * KW // 2:(kq + 1) * KW // 2, cs]),
                            preferred_element_type=f32)
                if kq == 0:
                    acc_s[gr, cs] = d + b_s[r, :]
                elif kq < KQ - 1:
                    acc_s[gr, cs] += d
                else:
                    g = acc_s[gr, cs] + d
                    z1 = _unpk(z1_s[hrws(p, mq * MB2, MB2), cs]).astype(f32)
                    h_s[mq * MB2 // 2:(mq + 1) * MB2 // 2, cs] = _pk((z1 * g).astype(bf16))
            return f

        def mm3_a(mq, t):
            def f():
                cs = slice(t * C, (t + 1) * C)
                acc_s[mq * MB2:(mq + 1) * MB2, FH + t * C:FH + (t + 1) * C] = jnp.dot(
                    _unpk(h_s[mq * MB2 // 2:(mq + 1) * MB2 // 2, :4 * C]), _unpk(wout_s[:2 * C, cs]),
                    preferred_element_type=f32)
            return f

        def mm3_b(mq):
            def f():
                d = jnp.dot(_unpk(h_s[mq * MB2 // 2:(mq + 1) * MB2 // 2, 4 * C:]), _unpk(wout_s[2 * C:, :]),
                            preferred_element_type=f32)
                acc_s[mq * MB2:(mq + 1) * MB2, FH:FH + D] += d
            return f

        def silu_piece(mq, i):
            def f():
                rs = slice(mq * MB2 + 16 * i, mq * MB2 + 16 * (i + 1))
                hg = 0.5 * acc_s[rs, FH:FH + D]
                gate_s[rws(p, mq * MB2 + 16 * i, 16), :] = hg * (1.0 + jnp.tanh(hg))
            return f

        main = []
        sides = []
        npq = (FH // C) * KQ
        for mq in range(MQ2):
            blk = [mm2(mq, n, kq) for n in range(FH // C) for kq in range(KQ)]
            if mq > 0:
                m3 = [mm3_a(mq - 1, t) for t in range(D // C)] + [mm3_b(mq - 1)]
                sides.append(([silu_piece(mq - 1, i) for i in range(MB2 // 16)],
                              len(main) + 12, len(main) + 20))
                blk = blk[:4] + m3 + blk[4:]
            main += blk
        main += [mm3_a(MQ2 - 1, t) for t in range(D // C)] + [mm3_b(MQ2 - 1)]
        total = (CG // 8) * NC * (NC + 1) // 2
        sides.append(([lambda: next(gen)] * total, 0, len(main)))
        _run_schedule(main, sides)
        for i in range(MB2 // 16):
            silu_piece(MQ2 - 1, i)()
        for _ in gen:
            pass

    def phase2(p, carry):
        cp_wsp(p).wait()
        pl.when(go_s[0] > 0)(functools.partial(phase2_body, p))
        return carry

    lax.fori_loop(0, NB, phase2, 0)

    def phase3_body(p):

        def idft(c, cb):
            def f():
                yt = jnp.dot(_unpk(zb_s[p * CPB + c, cb * C // 2:(cb + 1) * C // 2, :]), _unpk(wip_s[...]),
                             preferred_element_type=f32)
                y_s[c * C:(c + 1) * C, cb * C:(cb + 1) * C] = yt.T
            return f

        def comb_piece(i):
            def f():
                r = rws(p, 16 * i, 16)
                rs = slice(16 * i, 16 * (i + 1))
                y = y_s[rs, :] + kv_s[r, :].astype(f32) * d_ref[...].astype(f32)
                s = _unpk(xn_s[hrws(p, 16 * i, 16), :]).astype(f32) * y
                out_s[r, :] = (x_s[r, :].astype(f32) + s * gate_s[r, :]).astype(bf16)
            return f

        main = [idft(c, cb) for c in range(CPB) for cb in range(D // C)]
        nm = D // C
        sides = [([comb_piece(i) for i in range(C // 16)], nm, 2 * nm)]
        _run_schedule(main, sides)
        for i in range(C // 16, TB // 16):
            comb_piece(i)()

    def phase3(p, carry):
        pl.when(go_s[0] > 0)(functools.partial(phase3_body, p))
        cp_out(p).start()
        return carry

    lax.fori_loop(0, NB, phase3, 0)
    for p in range(NB):
        cp_out(p).wait()


@jax.jit
def pallas_recurrent_scan__ssm_conv_h3__mixer_gmlp__prompt_kernel(
    A_q: jax.Array,
    A_k: jax.Array,
    A_v: jax.Array,
    A_shift_k: jax.Array,
    A_ssm_k: jax.Array,
    A_ssm_D: jax.Array,
    B_x: jax.Array,
    B_w_in: jax.Array,
    B_w_sp: jax.Array,
    B_b_sp: jax.Array,
    B_w_out: jax.Array,
):
    del B_x
    f32, bf16 = jnp.float32, jnp.bfloat16
    wf, wi = _dft_mats()
    hbm = pl.BlockSpec(memory_space=pl.ANY)
    vmem = pl.BlockSpec(memory_space=pltpu.VMEM)
    out = pl.pallas_call(
        _kernel,
        out_shape=jax.ShapeDtypeStruct((S, D), bf16),
        in_specs=[hbm, hbm, hbm, vmem, hbm, vmem, hbm, hbm, vmem, hbm, vmem, vmem],
        out_specs=hbm,
        scratch_shapes=[
            pltpu.VMEM((S, D), bf16),
            pltpu.VMEM((S + HALO, D), bf16),
            pltpu.VMEM((S, D), bf16),
            pltpu.VMEM((NC, D // 2, C), jnp.uint32),
            pltpu.VMEM((S // 2, S), jnp.uint32),
            pltpu.VMEM((FH // 2, D), jnp.uint32),
            pltpu.VMEM((S // 2, D), jnp.uint32),
            pltpu.VMEM((S, D), bf16),
            pltpu.VMEM((S // 2, FH), jnp.uint32),
            pltpu.VMEM((S // 2, FH), jnp.uint32),
            pltpu.VMEM((NC, D, 2 * C), f32),
            pltpu.VMEM((NC, D, 2 * C), f32),
            pltpu.VMEM((S, C), f32),
            pltpu.VMEM((TB, F), f32),
            pltpu.VMEM((2, CPB, D // 2, C), jnp.uint32),
            pltpu.VMEM((NC, D // 2, 2 * C), jnp.uint32),
            pltpu.VMEM((TB // 2, FH), jnp.uint32),
            pltpu.VMEM((TB, D), f32),
            pltpu.VMEM((S, D), f32),
            pltpu.VMEM((D // 2, F), jnp.uint32),
            pltpu.VMEM((C // 2, 2 * C), jnp.uint32),
            pltpu.VMEM((C, C), jnp.uint32),
            pltpu.VMEM((TB, D), f32),
            pltpu.VMEM((S, D), bf16),
            pltpu.SMEM((1,), jnp.int32),
            pltpu.SemaphoreType.DMA((4, NB)),
            pltpu.SemaphoreType.DMA((NC,)),
            pltpu.SemaphoreType.DMA((3,)),
            pltpu.SemaphoreType.DMA((NB,)),
        ],
        compiler_params=pltpu.CompilerParams(vmem_limit_bytes=100 * 1024 * 1024),
    )(
        A_q.reshape(S, D), A_k.reshape(S, D), A_v.reshape(S, D),
        A_shift_k.T, A_ssm_k, A_ssm_D.reshape(1, D), B_w_in, B_w_sp,
        B_b_sp.reshape(1, S), B_w_out,
        jnp.asarray(wf, dtype=bf16), jnp.asarray(wi, dtype=bf16),
    )
    return out.reshape(1, S, D)
```

```python
import functools

import jax
import jax.numpy as jnp
import numpy as np
from jax import lax
import jax.experimental.pallas as pl
import jax.experimental.pallas.tpu as pltpu

S, D, F, FH, KS = 2048, 640, 1536, 768, 4
C = 128
NC = S // C
TB = 256
NB = S // TB
CPB = TB // C
CG = D // NB
HALO = 16
EPS = 1e-5


def _dft_mats():
    t = np.arange(C, dtype=np.float64)[:, None]
    w = 2.0 * np.pi * (np.arange(C, dtype=np.float64)[None, :] + 0.5) / (2 * C)
    fwd = np.concatenate([np.cos(w * t), -np.sin(w * t)], axis=1)
    inv = fwd.T / C
    return fwd.astype(np.float32), inv.astype(np.float32)


def _layernorm(x):
    m = jnp.mean(x, axis=-1, keepdims=True)
    xc = x - m
    v = jnp.mean(xc * xc, axis=-1, keepdims=True)
    return xc * lax.rsqrt(v + EPS)


def _gelu(x):
    c0 = np.float32(np.sqrt(2.0 / np.pi))
    c1 = np.float32(np.sqrt(2.0 / np.pi) * 0.044715)
    return (0.5 * x) * (1.0 + jnp.tanh(x * (c0 + c1 * (x * x))))


def _pk(v):
    return pltpu.bitcast(v, jnp.uint32)


def _unpk(u):
    return pltpu.bitcast(u, jnp.bfloat16)


def _run_schedule(main, sides):
    done = [0] * len(sides)
    for u, f in enumerate(main):
        f()
        for si, (pieces, u0, u1) in enumerate(sides):
            n = len(pieces)
            tgt = n if u >= u1 - 1 else max(0, (u - u0 + 1) * n // (u1 - u0))
            while done[si] < tgt:
                pieces[done[si]]()
                done[si] += 1


def _kernel(x_hbm, k_hbm, v_hbm, shk_ref, ssmk_hbm, d_ref, win_hbm, wsp_hbm, b_ref,
            wout_hbm, wf_ref, wi_ref, out_hbm,
            x_s, k_s, v_s, ssmk_s, wsp_s, wout_s, xn_s, z1_s, z2_s,
            u_s, kf_s, b_s, acc_s, kvt_s, zb_s, h_s, y_s, gate_s, winp_s, wfp_s, wip_s, kvb0_s, d_s, out_s, go_s, sem_in, sem_w, sem_out):
    f32, bf16 = jnp.float32, jnp.bfloat16

    u32 = jnp.uint32
    wsp_hbm, win_hbm = wsp_hbm.bitcast(u32), win_hbm.bitcast(u32)
    wout_hbm, ssmk_hbm = wout_hbm.bitcast(u32), ssmk_hbm.bitcast(u32)

    def rows(p):
        return pl.ds(pl.multiple_of(p * TB, TB), TB)

    def _cp(src, dst, i):
        return pltpu.make_async_copy(src, dst, sem_in.at[i])

    cp_x = [_cp(x_hbm.at[pl.ds(a, n)], x_s.at[pl.ds(a, n)], i)
            for i, (a, n) in enumerate([(0, TB), (TB, TB), (2 * TB, S - 2 * TB)])]
    cp_k = _cp(k_hbm, k_s.at[pl.ds(HALO, S)], 3)
    cp_v = _cp(v_hbm, v_s, 4)
    cp_ssmk = _cp(ssmk_hbm, ssmk_s, 5)
    WB = S // 8
    cp_wsp = [_cp(wsp_hbm.at[pl.ds(i * WB, WB)], wsp_s.at[pl.ds(i * WB, WB)], 6 + i) for i in range(4)]

    def cp_out(p):
        return pltpu.make_async_copy(out_s.at[rows(p)], out_hbm.at[rows(p)], sem_out.at[p])

    cp_win = [pltpu.make_async_copy(win_hbm.at[:, FH:], winp_s.at[:, :FH], sem_w.at[0]),
              pltpu.make_async_copy(win_hbm.at[:, :FH], winp_s.at[:, FH:], sem_w.at[2])]
    cp_wout = pltpu.make_async_copy(wout_hbm, wout_s, sem_w.at[1])

    cp_x[0].start()
    for cp in cp_win:
        cp.start()

    go_s[0] = 1
    k_s[pl.ds(0, HALO), :] = jnp.zeros((HALO, D), bf16)
    d_s[...] = jnp.broadcast_to(d_ref[...].astype(f32).reshape(1, D), (8, D))
    ball = b_ref[...].astype(f32).reshape(1, S)
    for c in range(NC):
        brow = ball[:, c * C:(c + 1) * C]
        b_s[c * C:(c + 1) * C, :] = jnp.broadcast_to(brow, (C, C)).T

    def rws(p, off, n):
        return pl.ds(pl.multiple_of(p * TB + off, n if n < 16 else 16), n)

    def hrws(p, off, n):
        return pl.ds(pl.multiple_of((p * TB + off) // 2, 8), n // 2)

    def ln_piece(p, i):
        def f():
            r = rws(p, 16 * i, 16)
            xn_s[hrws(p, 16 * i, 16), :] = _pk(_layernorm(x_s[r, :].astype(f32)).astype(bf16))
        return f

    CONV_N = 64

    def conv_piece(p, dst, i, t):
        def f():
            n = CONV_N
            cs = slice(t * C, (t + 1) * C)
            shk = shk_ref[:, cs].astype(f32)
            kwin = k_s[pl.ds(pl.multiple_of(p * TB + HALO + n * i - 8, 8), n + 8), cs].astype(f32)
            ksh = kwin[8:, :] * shk[0:1, :]
            for tau in range(1, KS):
                ksh = ksh + kwin[8 - tau:8 - tau + n, :] * shk[tau:tau + 1, :]
            r = rws(p, n * i, n)
            kv = ksh * v_s[r, cs].astype(f32)
            dst[n * i:n * (i + 1), cs] = kv
        return f

    def tr_piece(src, slot, c, t):
        def f():
            blk = src[c * C:(c + 1) * C, t * C:(t + 1) * C]
            kvt_s[slot, c, t * C // 2:(t + 1) * C // 2, :] = _pk(blk.T.astype(bf16))
        return f

    wfp_s[...] = _pk(wf_ref[...])
    wip_s[...] = _pk(wi_ref[...])

    kvt_s[...] = jnp.zeros((2, CPB, D // 2, C), jnp.uint32)
    cp_x[0].wait()
    cp_x[1].start()
    for i in range(TB // 16):
        ln_piece(0, i)()
    for cp in cp_win:
        cp.wait()
    for cp in [cp_x[2], cp_k, cp_v, cp_ssmk, cp_wout] + cp_wsp:
        cp.start()

    MB = 64
    MQ = TB // MB
    NG = 4 * C

    def phase1_body(p):
        pn = jnp.minimum(p + 1, NB - 1)

        def mm1_a(j, mq, t):
            def f():
                cs = slice(j * NG + t * C, j * NG + (t + 1) * C)
                d = jnp.dot(_unpk(xn_s[hrws(p, mq * MB, MB), :4 * C]), _unpk(winp_s[:2 * C, cs]),
                            preferred_element_type=f32)
                acc_s[mq * MB:(mq + 1) * MB, cs] = d
            return f

        def mm1_b(j, mq):
            def f():
                cs = slice(j * NG, (j + 1) * NG)
                d = jnp.dot(_unpk(xn_s[hrws(p, mq * MB, MB), 4 * C:]), _unpk(winp_s[2 * C:, cs]),
                            preferred_element_type=f32)
                acc_s[mq * MB:(mq + 1) * MB, cs] += d
            return f

        def gelu_piece(j, mq, t):
            def f():
                c0 = j * NG + t * C
                rs = slice(mq * MB, (mq + 1) * MB)
                z = _gelu(acc_s[rs, c0:c0 + C])
                if c0 < FH:
                    acc_s[rs, c0:c0 + C] = z
                else:
                    z1_s[hrws(p, mq * MB, MB), c0 - FH:c0 - FH + C] = _pk(z.astype(bf16))
            return f

        def ln2_piece(i):
            def f():
                z2 = acc_s[16 * i:16 * (i + 1), :FH]
                z2_s[hrws(p, 16 * i, 16), :] = _pk(_layernorm(z2).astype(bf16))
            return f

        main = []
        for j in range(F // NG):
            for mq in range(MQ):
                main += [mm1_a(j, mq, t) for t in range(NG // C)] + [mm1_b(j, mq)]
        n_mm = len(main)
        upb = NG // C + 1
        sides = []
        for b in range(3 * MQ):
            j, mq = divmod(b, MQ)
            if b + 1 < 3 * MQ:
                sides.append(([gelu_piece(j, mq, t) for t in range(NG // C)],
                              (b + 1) * upb, (b + 2) * upb))
        sides.append(([ln2_piece(i) for i in range(TB // 16)], 45, 60))
        sides.append(([ln_piece(pn, i) for i in range(TB // 16)], 10, 40))
        _run_schedule(main, sides)
        for t in range(NG // C):
            gelu_piece(F // NG - 1, MQ - 1, t)()

    def phase1(p, carry):
        pl.when(p == 0)(cp_x[1].wait)
        pl.when(p == 1)(cp_x[2].wait)
        pl.when(go_s[0] > 0)(functools.partial(phase1_body, p))
        return carry

    lax.fori_loop(0, NB, phase1, 0)

    def dft_unit(src, dst, blk, c, cb):
        def f():
            dst[blk * CPB + c, cb * C:(cb + 1) * C, :] = jnp.dot(
                _unpk(src(c, slice(cb * C // 2, (cb + 1) * C // 2))), _unpk(wfp_s[...]),
                preferred_element_type=f32)
        return f

    def u_units(blk, c):
        return [dft_unit(lambda c_, hr: kvt_s[0, c_, hr, :], u_s, blk, c, cb) for cb in range(D // C)]

    def phaseA_body(p):
        main = [dft_unit(lambda c_, hr: ssmk_s[hr, pl.ds(pl.multiple_of((p * CPB + c_) * C, C), C)], kf_s, p, c, cb)
                for c in range(CPB) for cb in range(D // C)]
        main += u_units(p, 0) + u_units(p, 1)
        hc = C // CONV_N
        sides = []
        for c in range(CPB):
            sides.append(([conv_piece(p, kvb0_s, i, t) for t in range(D // C) for i in range(c * hc, (c + 1) * hc)],
                          5 * c, 5 * c + 5))
            sides.append(([tr_piece(kvb0_s, 0, c, t) for t in range(D // C)], 5 * c + 2, 5 * c + 8))
        _run_schedule(main, sides)

    def phaseA(p, carry):
        pl.when(go_s[0] > 0)(functools.partial(phaseA_body, p))
        return carry

    cp_k.wait()
    cp_v.wait()
    cp_ssmk.wait()
    lax.fori_loop(0, NB, phaseA, 0)
    for t in range(D // C):
        dcol = jnp.broadcast_to(d_s[0:1, t * C:(t + 1) * C], (C, C)).T
        kf_s[0, t * C:(t + 1) * C, :C] += dcol
    cp_wout.wait()

    IB = 4

    lane = lax.broadcasted_iota(jnp.int32, (1, C), 1)
    sgn = (1 - 2 * (lane & 1)).astype(f32)

    def mac_gen(p):
        for g2 in range(CG // 16):
            prev = [None, None]
            for ib in range(0, NC, IB):
                res = []
                for half in range(2):
                    ch = pl.ds(pl.multiple_of(p * CG + g2 * 16 + half * 8, 8), 8)
                    ucache = {}
                    accr = [None] * IB
                    acci = [None] * IB
                    for m in range(ib + IB):
                        kr = kf_s[m, ch, :C]
                        ki = kf_s[m, ch, C:]
                        for q in range(IB):
                            j = ib + q - m
                            if j < 0:
                                continue
                            if j not in ucache:
                                ucache[j] = (u_s[j, ch, :C], u_s[j, ch, C:])
                            ur, ui = ucache[j]
                            pr = kr * ur - ki * ui
                            pi = kr * ui + ki * ur
                            accr[q] = pr if accr[q] is None else accr[q] + pr
                            acci[q] = pi if acci[q] is None else acci[q] + pi
                            yield
                    out = []
                    for q in range(IB):
                        if prev[half] is None:
                            out.append((accr[q], acci[q]))
                        else:
                            out.append((accr[q] - sgn * prev[half][1], acci[q] + sgn * prev[half][0]))
                        prev[half] = (accr[q], acci[q])
                    res.append(out)
                ro = pl.ds(pl.multiple_of((p * CG + g2 * 16) // 2, 8), 8)
                for q in range(IB):
                    for part in range(2):
                        v = jnp.concatenate([res[0][q][part], res[1][q][part]], axis=0)
                        zb_s[ib + q, ro, part * C:(part + 1) * C] = _pk(v.astype(bf16))

    MB2 = 128
    MQ2 = TB // MB2

    def phase2_body(p):
        KQ = 4
        KW = S // KQ
        gen = mac_gen(p)

        def mm2(mq, n, kq):
            def f():
                cs = slice(n * C, (n + 1) * C)
                r = rws(p, mq * MB2, MB2)
                gr = slice(mq * MB2, (mq + 1) * MB2)
                ks = slice(kq * KW, (kq + 1) * KW)
                d = jnp.dot(_unpk(wsp_s[hrws(p, mq * MB2, MB2), ks]), _unpk(z2_s[kq * KW // 2:(kq + 1) * KW // 2, cs]),
                            preferred_element_type=f32)
                if kq == 0:
                    acc_s[gr, cs] = d + b_s[r, :]
                elif kq < KQ - 1:
                    acc_s[gr, cs] += d
                else:
                    g = acc_s[gr, cs] + d
                    z1 = _unpk(z1_s[hrws(p, mq * MB2, MB2), cs]).astype(f32)
                    h_s[mq * MB2 // 2:(mq + 1) * MB2 // 2, cs] = _pk((z1 * g).astype(bf16))
            return f

        def mm3_a(mq, t):
            def f():
                cs = slice(t * C, (t + 1) * C)
                acc_s[mq * MB2:(mq + 1) * MB2, FH + t * C:FH + (t + 1) * C] = jnp.dot(
                    _unpk(h_s[mq * MB2 // 2:(mq + 1) * MB2 // 2, :4 * C]), _unpk(wout_s[:2 * C, cs]),
                    preferred_element_type=f32)
            return f

        def mm3_b(mq):
            def f():
                d = jnp.dot(_unpk(h_s[mq * MB2 // 2:(mq + 1) * MB2 // 2, 4 * C:]), _unpk(wout_s[2 * C:, :]),
                            preferred_element_type=f32)
                acc_s[mq * MB2:(mq + 1) * MB2, FH:FH + D] += d
            return f

        def silu_piece(mq, i):
            def f():
                rs = slice(mq * MB2 + 16 * i, mq * MB2 + 16 * (i + 1))
                hg = 0.5 * acc_s[rs, FH:FH + D]
                gate_s[rws(p, mq * MB2 + 16 * i, 16), :] = hg * (1.0 + jnp.tanh(hg))
            return f

        main = []
        sides = []
        npq = (FH // C) * KQ
        for mq in range(MQ2):
            blk = [mm2(mq, n, kq) for n in range(FH // C) for kq in range(KQ)]
            if mq > 0:
                m3 = [mm3_a(mq - 1, t) for t in range(D // C)] + [mm3_b(mq - 1)]
                sides.append(([silu_piece(mq - 1, i) for i in range(MB2 // 16)],
                              len(main) + 12, len(main) + 20))
                blk = blk[:4] + m3 + blk[4:]
            main += blk
        main += [mm3_a(MQ2 - 1, t) for t in range(D // C)] + [mm3_b(MQ2 - 1)]
        total = (CG // 8) * NC * (NC + 1) // 2
        sides.append(([lambda: next(gen)] * total, 0, len(main)))
        _run_schedule(main, sides)
        for i in range(MB2 // 16):
            silu_piece(MQ2 - 1, i)()
        for _ in gen:
            pass

    def phase2(p, carry):
        for i in range(4):
            pl.when(p == 2 * i)(cp_wsp[i].wait)
        pl.when(go_s[0] > 0)(functools.partial(phase2_body, p))
        return carry

    lax.fori_loop(0, NB, phase2, 0)

    def phase3_body(p):

        def idft(c, cb):
            def f():
                yt = jnp.dot(_unpk(zb_s[p * CPB + c, cb * C // 2:(cb + 1) * C // 2, :]), _unpk(wip_s[...]),
                             preferred_element_type=f32)
                y_s[c * C:(c + 1) * C, cb * C:(cb + 1) * C] = yt.T
            return f

        def comb_piece(i):
            def f():
                r = rws(p, 16 * i, 16)
                rs = slice(16 * i, 16 * (i + 1))
                y = y_s[rs, :]
                s = _unpk(xn_s[hrws(p, 16 * i, 16), :]).astype(f32) * y
                out_s[r, :] = (x_s[r, :].astype(f32) + s * gate_s[r, :]).astype(bf16)
            return f

        main = [idft(c, cb) for c in range(CPB) for cb in range(D // C)]
        nm = D // C
        sides = [([comb_piece(i) for i in range(C // 16)], nm, 2 * nm)]
        _run_schedule(main, sides)
        for i in range(C // 16, TB // 16):
            comb_piece(i)()

    def phase3(p, carry):
        pl.when(go_s[0] > 0)(functools.partial(phase3_body, p))
        cp_out(p).start()
        return carry

    lax.fori_loop(0, NB, phase3, 0)
    for p in range(NB):
        cp_out(p).wait()


@jax.jit
def pallas_recurrent_scan__ssm_conv_h3__mixer_gmlp__prompt_kernel(
    A_q: jax.Array,
    A_k: jax.Array,
    A_v: jax.Array,
    A_shift_k: jax.Array,
    A_ssm_k: jax.Array,
    A_ssm_D: jax.Array,
    B_x: jax.Array,
    B_w_in: jax.Array,
    B_w_sp: jax.Array,
    B_b_sp: jax.Array,
    B_w_out: jax.Array,
):
    del B_x
    f32, bf16 = jnp.float32, jnp.bfloat16
    wf, wi = _dft_mats()
    hbm = pl.BlockSpec(memory_space=pl.ANY)
    vmem = pl.BlockSpec(memory_space=pltpu.VMEM)
    out = pl.pallas_call(
        _kernel,
        out_shape=jax.ShapeDtypeStruct((S, D), bf16),
        in_specs=[hbm, hbm, hbm, vmem, hbm, vmem, hbm, hbm, vmem, hbm, vmem, vmem],
        out_specs=hbm,
        scratch_shapes=[
            pltpu.VMEM((S, D), bf16),
            pltpu.VMEM((S + HALO, D), bf16),
            pltpu.VMEM((S, D), bf16),
            pltpu.VMEM((D // 2, S), jnp.uint32),
            pltpu.VMEM((S // 2, S), jnp.uint32),
            pltpu.VMEM((FH // 2, D), jnp.uint32),
            pltpu.VMEM((S // 2, D), jnp.uint32),
            pltpu.VMEM((S // 2, FH), jnp.uint32),
            pltpu.VMEM((S // 2, FH), jnp.uint32),
            pltpu.VMEM((NC, D, 2 * C), f32),
            pltpu.VMEM((NC, D, 2 * C), f32),
            pltpu.VMEM((S, C), f32),
            pltpu.VMEM((TB, F), f32),
            pltpu.VMEM((2, CPB, D // 2, C), jnp.uint32),
            pltpu.VMEM((NC, D // 2, 2 * C), jnp.uint32),
            pltpu.VMEM((TB // 2, FH), jnp.uint32),
            pltpu.VMEM((TB, D), f32),
            pltpu.VMEM((S, D), f32),
            pltpu.VMEM((D // 2, F), jnp.uint32),
            pltpu.VMEM((C // 2, 2 * C), jnp.uint32),
            pltpu.VMEM((C, C), jnp.uint32),
            pltpu.VMEM((TB, D), f32),
            pltpu.VMEM((8, D), f32),
            pltpu.VMEM((S, D), bf16),
            pltpu.SMEM((1,), jnp.int32),
            pltpu.SemaphoreType.DMA((10,)),
            pltpu.SemaphoreType.DMA((3,)),
            pltpu.SemaphoreType.DMA((NB,)),
        ],
        compiler_params=pltpu.CompilerParams(vmem_limit_bytes=100 * 1024 * 1024),
    )(
        A_q.reshape(S, D), A_k.reshape(S, D), A_v.reshape(S, D),
        A_shift_k.T, A_ssm_k, A_ssm_D, B_w_in, B_w_sp,
        B_b_sp, B_w_out,
        jnp.asarray(wf, dtype=bf16), jnp.asarray(wi, dtype=bf16),
    )
    return out.reshape(1, S, D)
```
